```python
import os as _os
_os.environ.setdefault("JAX_PLATFORMS", "cpu")
import jax
import jax.numpy as jnp

def _softmax(x, axis=-1):
    return jax.nn.softmax(x, axis=axis)
def _gelu(x):
    return jax.nn.gelu(x, approximate=True)
def _silu(x):
    return jax.nn.silu(x)
def _sigmoid(x):
    return jax.nn.sigmoid(x)
def _layernorm(x, axis=-1, eps=1e-5):
    m = jnp.mean(x, axis=axis, keepdims=True)
    v = jnp.var(x, axis=axis, keepdims=True)
    return (x - m) / jnp.sqrt(v + eps)
def _scatter_add(tgt, idx, src, axis=0):
    return tgt.at[idx].add(src)
def _segment_sum(src, seg, n):
    return jax.ops.segment_sum(src, seg, n)
class _Rng:
    def __init__(self, key):
        self._k = key
    def _next(self):
        self._k, sub = jax.random.split(self._k)
        return sub
    def normal(self, shape):
        return jax.random.normal(self._next(), shape, dtype=jnp.bfloat16)
    def randint(self, lo, hi, shape):
        return jax.random.randint(self._next(), shape, lo, hi, dtype=jnp.int32)
    def uniform(self, shape, lo=0.0, hi=1.0):
        return jax.random.uniform(self._next(), shape, jnp.bfloat16, lo, hi)
    def permutation(self, n):
        return jax.random.permutation(self._next(), n)


kernel_name = 'parallel_sum__sliding_local_dilated__glu_gated_reglu__prompt'

def setup_inputs():
    _rng = _Rng(jax.random.key(int.from_bytes(__import__("os").urandom(4), "little")))
    _w = (lambda a: (lambda t: t.astype(jnp.bfloat16) if jnp.issubdtype(t.dtype, jnp.floating) else t)(jnp.asarray(a)))
    def _A_setup():
        B, S, D = 1, 2048, 576
        return {
            "x": _w((lambda *s: _rng.normal(s) * 0.05)(B, S, D)),
            "wqkv": _w((lambda *s: _rng.normal(s) * 0.05)(D, 3 * D)),
            "wo": _w((lambda *s: _rng.normal(s) * 0.05)(D, D)),
        }
    _A_in = _A_setup()

    def _B_setup():
        B, S, D, F = 1, 2048, 576, 4608
        return {
            "x": _w((lambda *s: _rng.normal(s) * 0.05)(B, S, D)),
            "W_gate": _w((lambda *s: _rng.normal(s) * 0.1)(D, F) * (2.0 / D) ** 0.5),
            "W_up": _w((lambda *s: _rng.normal(s) * 0.1)(D, F) * (2.0 / D) ** 0.5),
            "W_down": _w((lambda *s: _rng.normal(s) * 0.1)(F, D) * (1.0 / F) ** 0.5),
        }
    _B_in = _B_setup()

    return {
        "A_x": _A_in["x"],
        "A_wqkv": _A_in["wqkv"],
        "A_wo": _A_in["wo"],
        "B_x": _B_in["x"],
        "B_W_gate": _B_in["W_gate"],
        "B_W_up": _B_in["W_up"],
        "B_W_down": _B_in["W_down"],
    }

def reference(A_x, A_wqkv, A_wo, B_x, B_W_gate, B_W_up, B_W_down):
    def _A_ref(x, wqkv, wo):
        B, S, D = x.shape
        H = 32; Dh = D // H
        W, dil = 8, 2
        qkv = (lambda x, *d: x.transpose(*d))((x @ wqkv).reshape(B, S, 3, H, Dh), 2, 0, 3, 1, 4)
        q, k, v = qkv[0], qkv[1], qkv[2]
        scale = Dh ** -0.5
        pos = jnp.arange(S)
        off = jnp.arange(W) * dil
        idx = pos[:, None] - off[None, :]
        mask = idx >= 0
        idx_c = jnp.where(mask, idx, 0).reshape(-1)
        kg = k[:, :, idx_c, :].reshape(B, H, S, W, Dh)
        vg = v[:, :, idx_c, :].reshape(B, H, S, W, Dh)
        logits = jnp.einsum("bhsd,bhswd->bhsw", q, kg) * scale
        logits = jnp.where(mask[None, None, :, :], logits, -1e9)
        attn = _softmax(logits, axis=-1)
        o = jnp.einsum("bhsw,bhswd->bhsd", attn, vg)
        return (lambda x, *d: x.transpose(*d))(o, 0, 2, 1, 3).reshape(B, S, D) @ wo

    def _B_ref(x, W_gate, W_up, W_down):
        gate = jnp.einsum("bsd,df->bsf", x, W_gate)
        up = jnp.einsum("bsd,df->bsf", x, W_up)
        gate = gate * (lambda x, dt: x.astype(dt))(gate > 0, gate.dtype)
        h = gate * up
        return jnp.einsum("bsf,fd->bsd", h, W_down)

    x = A_x
    xn = _layernorm(x, axis=-1)
    return x + _A_ref(xn, A_wqkv, A_wo) + _B_ref(xn, B_W_gate, B_W_up, B_W_down)
```

```python
import functools
import itertools

import jax
import jax.numpy as jnp
import numpy as np
from jax import lax
from jax.experimental import pallas as pl
from jax.experimental.pallas import tpu as pltpu

F32 = jnp.float32
BF16 = jnp.bfloat16
U32 = jnp.uint32

S, D, F = 2048, 576, 4608
H, DH, WIN, DIL = 32, 18, 8, 2
T = 128
GS = 4 * T
NG = S // GS
HG = H // 8
HR = 8 * DH
DB = D // 4
KU = 32
QUADS = ((0, 0), (0, 1), (1, 0), (1, 1))


def _nn(a, b):
    return jnp.dot(a, b, preferred_element_type=F32)


def _nt(a, b):
    return lax.dot_general(a, b, (((1,), (1,)), ((), ())), preferred_element_type=F32)


def _un(v):
    return pltpu.bitcast(v, BF16)


def _strassen(p, q):
    return {
        "m1": ({(0, p): 1, (1, q): 1}, {(p, 0): 1, (q, 1): 1}),
        "m2": ({(1, p): 1, (1, q): 1}, {(p, 0): 1}),
        "m4": ({(1, q): 1}, {(q, 0): 1, (p, 0): -1}),
        "m3": ({(0, p): 1}, {(p, 1): 1, (q, 1): -1}),
        "m5": ({(0, p): 1, (0, q): 1}, {(q, 1): 1}),
        "m6": ({(1, p): 1, (0, p): -1}, {(p, 0): 1, (p, 1): 1}),
        "m7": ({(0, q): 1, (1, q): -1}, {(q, 0): 1, (q, 1): 1}),
    }


def _strassen_swapped(p, q):
    return {
        "x": ({(0, p): 1, (1, q): 1}, {(p, 1): 1, (q, 0): 1}),
        "m2": ({(1, p): -1, (1, q): -1}, {(p, 1): 1}),
        "m3": ({(1, q): 1}, {(q, 1): 1, (p, 1): -1}),
        "m4": ({(0, p): 1}, {(p, 0): 1, (q, 0): -1}),
        "m5": ({(0, p): -1, (0, q): -1}, {(q, 0): 1}),
        "c21": ({(1, p): 1, (0, p): -1}, {(p, 0): 1, (p, 1): 1}),
        "c12": ({(0, q): 1, (1, q): -1}, {(q, 0): 1, (q, 1): 1}),
    }


def _plain(k):
    return {name: ({(i, k): 1}, {(k, j): 1}) for name, (i, j) in zip(("m7", "c12", "c21", "m6"), QUADS)}


def _single(k, variant):
    a0, a1, both = {(0, k): 1}, {(1, k): -1}, {(0, k): 1, (1, k): 1}
    b0, b1 = {(k, 0): 1}, {(k, 1): 1}
    half, diff = {(0, k): .5, (1, k): .5}, {(0, k): .5, (1, k): -.5}
    return (
        {"e1": (a1, b0), "e2": (a1, b1), "m7": (both, {(k, 0): 1, (k, 1): 1}), "m5": (both, b1)},
        {"e1": (a0, b0), "e2": (a0, b1), "m6": (both, {(k, 0): 1, (k, 1): 1}), "m2": (both, b0)},
        {"e1": (diff, b0), "e2": (diff, b1), "m4": (half, b0), "m3": (half, b1)},
        {"e1": (a1, b0), "e2": (a0, b1), "m1": (both, b1), "m7": (both, {(k, 0): 1, (k, 1): -1})},
    )[variant]


OUTS = {
    "m1": {(0, 0): 1, (1, 1): 1}, "m2": {(1, 0): 1, (1, 1): -1}, "m4": {(0, 0): 1, (1, 0): 1},
    "m3": {(0, 1): 1, (1, 1): 1}, "m5": {(0, 1): 1, (0, 0): -1}, "m6": {(1, 1): 1}, "m7": {(0, 0): 1},
    "c12": {(0, 1): 1}, "c21": {(1, 0): 1}, "x": {(0, 1): 1, (1, 0): 1},
    "e1": {(0, 0): 1, (1, 0): -1}, "e2": {(0, 1): 1, (1, 1): -1},
}


def _merge(parts):
    return [(out, [p[name] for p in parts if name in p])
            for name, out in OUTS.items() if any(name in p for p in parts)]


def _inner_scheme(n):
    if n <= 4:
        return _merge([_plain(k) for k in range(n)])
    if n % 2 == 0:
        return _merge([_strassen(k, k + n // 2) for k in range(n // 2)])
    assert n == 9
    return _merge([_strassen(k, k + 3) for k in range(3)] + [_single(6 + v, v) for v in range(3)])


def _two_level(outer, inner):
    return [(out, terms, inner(len(terms))) for out, terms in outer]


SCHEMES = {
    65: _two_level(_merge([_strassen(k, k + 8) for k in range(8)]) + _merge([_plain(16), _plain(17)]), _inner_scheme),
    61: _two_level(_merge([_strassen(k, k + 6) for k in range(6)] + [_strassen_swapped(12 + k, 14 + k) for k in range(2)]
                          + [_plain(16), _plain(17)]), _inner_scheme),
    59: _two_level(_merge([_strassen(k, k + 7) for k in range(7)] + [_single(14 + v, v) for v in range(4)]),
                   _inner_scheme),
}
DOWN = _two_level(_merge([_strassen(0, 2), _strassen(1, 3)]), lambda n: _merge([_strassen(0, 1)]))


def _lin(pairs):
    pairs = sorted(pairs, key=lambda p: p[0] < 0)
    scale = abs(pairs[0][0])
    v = pairs[0][1] if pairs[0][0] > 0 else -pairs[0][1]
    for c, t in pairs[1:]:
        v = v + t if c > 0 else v - t
    return v if scale == 1 else v * scale


def _operands(scheme, side, blk):
    blk = functools.cache(blk)

    @functools.cache
    def mid(o, a, u):
        form = scheme[o][1][u][side]
        return _lin([(c, blk(2 * key[side] + a, key[1 - side])) for key, c in form.items()])

    def operand(o, r):
        return [_lin([(c, mid(o, key[side], key[1 - side])) for key, c in term[side].items()])
                for term in scheme[o][2][r][1]]
    return operand


class Sums:
    def __init__(self, scheme):
        self.scheme, self.part = scheme, {}

    def add(self, o, r, m):
        for ab, c in self.scheme[o][2][r][0].items():
            old = self.part.get((o, ab))
            self.part[o, ab] = _lin([(c, m)] if old is None else [(1, old), (c, m)])

    def result(self, i, j):
        return _lin([(out[i // 2, j // 2], self.part[o, (i % 2, j % 2)])
                     for o, (out, _, _) in reversed(list(enumerate(self.scheme))) if (i // 2, j // 2) in out])


def _rounds(scheme):
    rounds, rest, last = [], [], []
    for o, (_, _, inner) in enumerate(scheme):
        ids = [(o, r) for r in range(len(inner))]
        if len(ids) == 4:
            last.append(ids)
            continue
        rounds.append(ids[:4])
        rest += ids[4:]
        while len(rest) >= 4:
            rounds.append(rest[:4])
            rest = rest[4:]
    last = [p for ps in zip(*last) for p in ps]
    rounds += [[p] for p in rest]
    return rounds + [last[i:i + 4] for i in range(0, len(last), 4)]


def _interleave(*streams):
    order = sorted(((i + .5) / n, k) for k, (_, n) in enumerate(streams) for i in range(n))
    for _, k in order:
        next(streams[k][0])


def make_kernel(nch=9, flags=None, sch=61, keep_acc=True, scopes=False, early=2,
                ggs=((0, 1), (2, 3)), dgs=((0, 1), (2, 3)), fine=True):
    GU = SCHEMES[sch]
    GU_IDS = {p: i for i, p in enumerate((o, r) for o in range(len(GU)) for r in range(len(GU[o][2])))}
    GU_UNITS = [[(o, r) for r in range(len(i))] for o, (_, _, i) in enumerate(GU) if len(i) > 4]
    GU_UNITS += [[(o, r) for r in range(4) for o, (_, _, i) in enumerate(GU)
                  if len(i) == 4 and next(iter(i[r][0]))[0] == a] for a in range(2)]
    NR = len(GU_UNITS)
    W_PIECES = ((0, 256), (256, 256), (512, 512), (1024, 1024), (2048, F - 2048))
    nblk = min(NG, (2 * nch - 2) // 4)

    def kernel(xT_hbm, wqkv_hbm, wo_hbm, wg_hbm, wu_hbm, wdT_hbm, outT_hbm,
               x_v, wqkv_v, wo_v, w_v, out_v, xc, acc, wqkvT, woT, qkv, oT,
               sem_x, sem_a, sem_w, sem_o):
        def x_copy(g):
            return pltpu.make_async_copy(xT_hbm.at[:, pl.ds(g * GS, GS)], x_v[g], sem_x.at[g])

        def w_copy(i, piece):
            src = (wg_hbm, wu_hbm, wdT_hbm)[i]
            return pltpu.make_async_copy(src.at[:, pl.ds(*W_PIECES[piece])], w_v[i][piece], sem_w.at[3 * piece + i])

        def w_load(i, rows, c, n):
            piece = max(p for p, (a, _) in enumerate(W_PIECES) if a <= c)
            c -= W_PIECES[piece][0]
            return w_v[i][piece][rows, c:c + n]

        def a_copy(i):
            src, dst = ((wqkv_hbm, wqkv_v), (wo_hbm, wo_v))[i]
            return pltpu.make_async_copy(src, dst, sem_a.at[i])

        def o_copy(g):
            return pltpu.make_async_copy(out_v[g], outT_hbm.at[:, pl.ds(g * GS, GS)], sem_o.at[g])

        def put(ref, idx, v, keep=True):
            if keep:
                pltpu.store(ref.at[idx], v, mask=jnp.ones(v.shape, jnp.bool_))
            else:
                ref[idx] = v

        xnT = {}

        def normalise(g):
            xs = []
            for t in range(0, 4, 2):
                xf = x_v[g][:, t * T:(t + 2) * T].astype(F32)
                xm = xf - jnp.sum(xf, axis=0, keepdims=True) * (1.0 / D)
                var = jnp.sum(xm * xm, axis=0, keepdims=True) * (1.0 / D)
                xn = xm * lax.rsqrt(var + 1e-5)
                xs += [xn[:, :T], xn[:, T:]]
            for t in range(4):
                xnT[g, t] = xs[t].astype(BF16)
            operand = _operands(GU, 0, lambda q, k: xs[q][k * KU:(k + 1) * KU])
            for p in itertools.chain(*GU_UNITS):
                units = operand(*p)
                units += [jnp.zeros_like(units[0])] * (4 - len(units))
                v = jnp.concatenate(units, axis=0).astype(BF16).T
                put(xc[g][p[0]], (p[1],), pltpu.bitcast(v, U32))

        @functools.cache
        def gu_weights(n):
            wide = functools.cache(lambda i, k: w_load(i, slice(k * KU, (k + 1) * KU), 2 * n * T, 2 * T).astype(F32))
            operand = _operands(GU, 1, lambda m, k: wide(m // 2, k)[:, m % 2 * T:(m % 2 + 1) * T])
            return functools.cache(lambda p: jnp.concatenate(operand(*p), axis=0).astype(BF16))

        hid = {}

        def gate_up(n, gs):
            sums = {g: Sums(GU) for g in gs}
            for unit in GU_UNITS[:-2]:
                for g in gs:
                    products(n, g, unit, sums[g])
                    yield
            for g in gs:
                for a, unit in enumerate(GU_UNITS[-2:]):
                    products(n, g, unit, sums[g])
                    for q in (a, a + 2):
                        for e in range(2):
                            hid[2 * n + e, q, g] = (jnp.maximum(sums[g].result(q, e), 0.0)
                                                    * sums[g].result(q, e + 2))
                    yield

        def products(n, g, unit, sums):
            for p in unit:
                w = gu_weights(n)(p)
                sums.add(*p, _nn(_un(xc[g][p[0]][p[1], :, :w.shape[0]]), w))

        @functools.cache
        def down_weights(j):
            wide = functools.cache(lambda d, f: w_load(2, slice(d * DB, (d + 1) * DB), (4 * j + 2 * f) * T, 2 * T).astype(F32))
            operand = _operands(DOWN, 0, lambda d, f: wide(d, f // 2)[:, f % 2 * T:(f % 2 + 1) * T])
            return functools.cache(lambda p: operand(*p)[0].astype(BF16))

        def down(js, gs):
            operand = {(j, g): _operands(DOWN, 1, lambda q, f, j=j, g=g: hid[4 * j + f, q, g]) for j in js for g in gs}
            for o in range(7):
                for g in gs:
                    idx = (g, 7 * o)
                    for r in range(7):
                        w = [down_weights(j)((o, r)) for j in js]
                        h = [operand[j, g](o, r)[0].astype(BF16) for j in js]
                        m = functools.reduce(lambda a, c: a + c, [_nt(a, c) for a, c in zip(w, h)])
                        put(acc[g][o], (r,), m if js[0] == 0 else m + acc[g][o][r], keep_acc)
                    yield

        resid = {}

        def finish(j, g):
            operand = _operands(DOWN, 1, lambda q, f: hid[4 * j + f, q, g])
            sums = Sums(DOWN)
            for o in range(7):
                for r in range(7):
                    m = _nt(down_weights(j)((o, r)), operand(o, r)[0].astype(BF16))
                    sums.add(o, r, m + acc[g][o][r])
                if o == 6:
                    for d in range(4):
                        v = [sums.result(d, q) + resid[min(g, nblk - 1), d, q] for q in range(4)]
                        out_v[g][d * DB:(d + 1) * DB, :] = jnp.concatenate(v, axis=1).astype(BF16)
                    o_copy(g).start()
                yield

        def transpose_into(dst, src):
            for n0 in range(0, src.shape[1], T):
                nw = min(T, src.shape[1] - n0)
                for k0 in range(0, D, T):
                    kw = min(T, D - k0)
                    put(dst, (pl.ds(n0 // 2, nw // 2), pl.ds(k0, kw)),
                        pltpu.bitcast(src[k0:k0 + kw, n0:n0 + nw].T, U32))

        halo = {}

        def attention(b, hg):
            s = (b * HG + hg) % 2
            lane = lax.broadcasted_iota(jnp.int32, (8, T), 1)

            def project(part, t):
                w = _un(wqkvT[(part * D + hg * HR) // 2:(part * D + hg * HR + HR) // 2, :])
                qkv[hg][part][t][...] = _nn(w, xnT[b, t])

            def rows(part, t, d):
                return qkv[hg][part][t][pl.ds(d, 8, stride=DH), :]

            def shifted(part, t, d):
                cur = rows(part, t, d)
                if t > 0:
                    prev = rows(part, t - 1, d)
                elif b > 0:
                    prev = halo[hg, part, d]
                else:
                    prev = jnp.broadcast_to(cur[:, :1], cur.shape)
                if t == 3:
                    halo[hg, part, d] = cur
                return [cur] + [pltpu.roll(jnp.where(lane >= T - DIL * w, prev, cur), DIL * w, 1)
                                for w in range(1, WIN)]
            for t in range(4):
                project(0, t)
                yield
                project(1, t)
                lg = None
                for d in range(DH):
                    q = rows(0, t, d)
                    p = [q * k for k in shifted(1, t, d)]
                    lg = p if lg is None else [a + c for a, c in zip(lg, p)]
                lg = [a * (DH ** -0.5) for a in lg]
                if b == 0 and t == 0:
                    lg = [lg[0]] + [jnp.where(lane >= DIL * w, lg[w], -1e9) for w in range(1, WIN)]
                mx = functools.reduce(jnp.maximum, lg)
                e = [jnp.exp(a - mx) for a in lg]
                inv = 1.0 / functools.reduce(lambda a, c: a + c, e)
                probs = [a * inv for a in e]
                yield
                project(2, t)
                for d in range(DH):
                    o = functools.reduce(lambda a, c: a + c, [a * c for a, c in zip(probs, shifted(2, t, d))])
                    oT[b][t][pl.ds(hg * HR + d, 8, stride=DH), :] = o
                yield

        def out_proj(b, ts):
            for t in ts:
                o = oT[b][t][...].astype(BF16)
                for d in range(4):
                    resid[b, d, t] = (_nn(_un(woT[d * DB // 2:(d + 1) * DB // 2, :]), o)
                                      + x_v[b][d * DB:(d + 1) * DB, t * T:(t + 1) * T].astype(F32))
                    yield

        def start(*cs):
            for c in cs:
                c.start()

        nw = [0]

        def wait(*cs):
            nw[0] += 1
            with jax.named_scope(f"wait{nw[0]}"):
                for c in cs:
                    c.wait()

        stages = [
            lambda: [x_copy(0)],
            lambda: [w_copy(0, 0), w_copy(1, 0)],
            lambda: [w_copy(0, 1), w_copy(1, 1), x_copy(1)],
            lambda: [x_copy(2), x_copy(3)],
            lambda: [a_copy(0), w_copy(2, 0), w_copy(2, 1), w_copy(0, 2), w_copy(1, 2)],
            lambda: [a_copy(1), w_copy(2, 2)] + [w_copy(i, 3) for i in range(3)],
            lambda: [w_copy(i, 4) for i in range(3)],
            lambda: [],
        ]
        start(*stages[0](), *stages[1]())
        if early == 0:
            start(*stages[2]())
        wait(*stages[0]())
        if early == 1:
            start(*stages[2]())
        normalise(0)
        wait(*stages[1]())
        if early == 2:
            start(*stages[2]())
        _interleave((gate_up(0, [0]), NR))
        wait(*stages[2]())
        start(*stages[3]())
        normalise(1)
        _interleave((gate_up(1, [0, 1]), 2 * NR), (gate_up(0, [1]), NR))
        wait(*stages[3]())
        start(*stages[4]())
        for g in (2, 3):
            normalise(g)
            _interleave((gate_up(0, [g]), NR), (gate_up(1, [g]), NR))
        wait(*stages[4]())
        start(*stages[5]())
        transpose_into(wqkvT, wqkv_v)
        for n in range(2, 2 * nch):
            if n == 4:
                wait(*stages[5]())
                start(*stages[6]())
                transpose_into(woT, wo_v)
            if n == min(8, 2 * nch - 1):
                wait(*stages[6]())
            if n % 2 == 0:
                dn = itertools.chain(*[down([n // 2 - 1], gs) for gs in dgs])
            streams = [(itertools.chain(*[gate_up(n, gs) for gs in ggs]), NG * NR), (dn, 14)]
            b, hg = divmod(n - 2, HG)
            if b < nblk:
                streams.append((attention(b, hg), 12))
                if b > 0:
                    streams.append((out_proj(b - 1, [hg]), 4))
            _interleave(*streams)
        if nblk > 1:
            _interleave((finish(nch - 1, 0), 7))
        _interleave((out_proj(nblk - 1, range(4)), 16))
        for g in range(1 if nblk > 1 else 0, NG):
            _interleave((finish(nch - 1, g), 7))
        wait(*[o_copy(g) for g in range(NG)])

    scratch = [
        [pltpu.VMEM((D, GS), BF16)] * NG,
        pltpu.VMEM((D, 3 * D), BF16),
        pltpu.VMEM((D, D), BF16),
        [[pltpu.VMEM((D, n), BF16) for _, n in W_PIECES]] * 3,
        [pltpu.VMEM((D, GS), BF16)] * NG,
        [[pltpu.VMEM((len(i), T // 2, T), U32) for _, _, i in GU]] * NG,
        [[pltpu.VMEM((7, DB, T), F32)] * 7] * NG,
        pltpu.VMEM((3 * D // 2, D), U32),
        pltpu.VMEM((D // 2, D), U32),
        [[[pltpu.VMEM((HR, T), F32)] * 4] * 3] * HG,
        [[pltpu.VMEM((D, T), F32)] * 4] * NG,
        pltpu.SemaphoreType.DMA((NG,)),
        pltpu.SemaphoreType.DMA((2,)),
        pltpu.SemaphoreType.DMA((3 * len(W_PIECES),)),
        pltpu.SemaphoreType.DMA((NG,)),
    ]

    def fn(A_x, A_wqkv, A_wo, B_x, B_W_gate, B_W_up, B_W_down):
        hbm = pl.BlockSpec(memory_space=pltpu.HBM)
        outT = pl.pallas_call(
            kernel,
            in_specs=[hbm] * 6,
            out_specs=hbm,
            out_shape=jax.ShapeDtypeStruct((D, S), BF16),
            scratch_shapes=scratch,
            compiler_params=pltpu.CompilerParams(vmem_limit_bytes=124 << 20, flags=flags),
            name="fusedblk",
        )(A_x.reshape(S, D).T, A_wqkv, A_wo, B_W_gate, B_W_up, B_W_down.T)
        return outT.T.reshape(1, S, D)
    return fn


@jax.jit
def pallas_parallel_sum__sliding_local_dilated__glu_gated_reglu__prompt_kernel(
    A_x, A_wqkv, A_wo, B_x, B_W_gate, B_W_up, B_W_down
):
    return make_kernel()(A_x, A_wqkv, A_wo, B_x, B_W_gate, B_W_up, B_W_down)
```

```python
import functools
import itertools

import jax
import jax.numpy as jnp
from jax import lax
from jax.experimental import pallas as pl
from jax.experimental.pallas import tpu as pltpu

F32, BF16, U32 = jnp.float32, jnp.bfloat16, jnp.uint32

S, D, F = 2048, 576, 4608
DH, WIN, DIL = 18, 8, 2
T = 128
GS = 4 * T
NG = S // GS
DB = D // 4
NSET = F // (2 * T)
DIMS = 3
W_PIECES = ((0, 256), (256, 256), (512, 256), (768, 256), (1024, 1024), (2048, F - 2048))
QUADS = ((0, 0), (0, 1), (1, 0), (1, 1))


OUTS = {
    "m1": {(0, 0): 1, (1, 1): 1}, "m2": {(1, 0): 1, (1, 1): -1}, "m4": {(0, 0): 1, (1, 0): 1},
    "m3": {(0, 1): 1, (1, 1): 1}, "m5": {(0, 1): 1, (0, 0): -1}, "m6": {(1, 1): 1}, "m7": {(0, 0): 1},
    "c12": {(0, 1): 1}, "c21": {(1, 0): 1}, "x": {(0, 1): 1, (1, 0): 1},
    "e1": {(0, 0): 1, (1, 0): -1}, "e2": {(0, 1): 1, (1, 1): -1},
}


def _strassen(p, q):
    return {
        "m1": ({(0, p): 1, (1, q): 1}, {(0, p): 1, (1, q): 1}),
        "m2": ({(1, p): 1, (1, q): 1}, {(0, p): 1}),
        "m4": ({(1, q): 1}, {(0, q): 1, (0, p): -1}),
        "m3": ({(0, p): 1}, {(1, p): 1, (1, q): -1}),
        "m5": ({(0, p): 1, (0, q): 1}, {(1, q): 1}),
        "m6": ({(1, p): 1, (0, p): -1}, {(0, p): 1, (1, p): 1}),
        "m7": ({(0, q): 1, (1, q): -1}, {(0, q): 1, (1, q): 1}),
    }


def _strassen_mirrored(p, q):
    return {
        "x": ({(0, p): 1, (1, q): 1}, {(1, p): 1, (0, q): 1}),
        "m2": ({(1, p): -1, (1, q): -1}, {(1, p): 1}),
        "m3": ({(1, q): 1}, {(1, q): 1, (1, p): -1}),
        "m4": ({(0, p): 1}, {(0, p): 1, (0, q): -1}),
        "m5": ({(0, p): -1, (0, q): -1}, {(0, q): 1}),
        "c21": ({(1, p): 1, (0, p): -1}, {(0, p): 1, (1, p): 1}),
        "c12": ({(0, q): 1, (1, q): -1}, {(0, q): 1, (1, q): 1}),
    }


def _plain(k):
    return {name: ({(i, k): 1}, {(j, k): 1}) for name, (i, j) in zip(("m7", "c12", "c21", "m6"), QUADS)}


def _single(k, variant):
    u0, u1, n1 = {(0, k): 1}, {(1, k): 1}, {(1, k): -1}
    add, sub = {(0, k): 1, (1, k): 1}, {(0, k): 1, (1, k): -1}
    half_add, half_sub = {(0, k): .5, (1, k): .5}, {(0, k): .5, (1, k): -.5}
    return (
        {"e1": (n1, u0), "e2": (n1, u1), "m7": (add, add), "m5": (add, u1)},
        {"e1": (u0, u0), "e2": (u0, u1), "m6": (add, add), "m2": (add, u0)},
        {"e1": (half_sub, u0), "e2": (half_sub, u1), "m4": (half_add, u0), "m3": (half_add, u1)},
        {"e1": (n1, u0), "e2": (u0, u1), "m1": (add, u1), "m7": (add, sub)},
    )[variant]


def _merge(parts):
    return [(out, [p[name] for p in parts if name in p])
            for name, out in OUTS.items() if any(name in p for p in parts)]


def _two_levels(outer):
    scheme = []
    for o, (out, terms) in enumerate(outer):
        n = len(terms)
        if o >= 7:
            inner = _merge([_plain(u) for u in range(n)])
        elif n == 5:
            inner = _merge([_strassen(0, 2), _single(3, 0), _single(4, 1), _single(1, 2)])
        elif n == 3:
            cut = lambda term: tuple({key: c for key, c in form.items() if key[1] < 3} for form in term)
            inner = [(ab, [t for t in map(cut, ts) if all(t)])
                     for ab, ts in _merge([_strassen(0, 3), _strassen(1, 2)])]
        else:
            inner = _merge([_strassen(u, u + n // 2) for u in range(n // 2)])
        if 3 <= o < 7:
            inner = [({(a, 1 - b): c for (a, b), c in ab.items()},
                      [(left, {(1 - b, u): c for (b, u), c in right.items()}) for left, right in ts])
                     for ab, ts in inner]
        scheme.append((out, terms, inner))
    return scheme


def _pair(start, size):
    return (start, size), (start + 2 * T, size)


LONE = ((224, 32), (480, 32), (512, 32), (544, 32), (512, 64))
ONE = _merge([_strassen(*_pair(0, 64)), _strassen(*_pair(64, 64)), _strassen_mirrored(*_pair(128, 64)),
              _plain(LONE[4]), _strassen(*_pair(192, 64))])
OUTPUT = _two_levels(ONE)
INPUT = _two_levels(_merge([_strassen(*_pair(0, 96)), _strassen(*_pair(96, 32)), _strassen(*_pair(128, 96))]
                           + [_single(LONE[v], v) for v in range(4)]))
DOWN = _two_levels(_merge([_strassen(0, 2), _strassen(1, 3)]))
INPUT_ORDER, OUTPUT_ORDER = (1, 5, 3, 0, 4, 2, 6), (3, 2, 0, 1, 5, 4, 6)


def _closing(scheme, a, b):
    return [(o, r) for o in range(7, len(scheme)) for r in range(4) if (a, b) in scheme[o][2][r][0]]


def _total(vs):
    vs = list(vs)
    while len(vs) > 1:
        vs = [a + b for a, b in zip(vs[::2], vs[1::2])] + vs[len(vs) // 2 * 2:]
    return vs[0]


def _signed(pairs):
    first = next((i for i, (c, _) in enumerate(pairs) if c > 0), 0)
    scale, v = pairs[first]
    for c, t in pairs[:first] + pairs[first + 1:]:
        v = v + t if c == scale else v - t
    return scale, v


def _lin(pairs):
    c, v = _signed(pairs)
    return v if c == 1 else v * c


class Operands:
    def __init__(self, side, block, nested=False):
        self.side, self.block, self.nested = side, functools.cache(block), nested

    def blocks(self, term, a):
        return [(c, self.block(2 * i + a, k)) for (i, k), c in term[self.side].items()]

    def one_level(self, o, a):
        return [_lin(self.blocks(term, a)) for term in ONE[o][1]]

    def two_levels(self, scheme, o, r):
        slices = []
        for term in scheme[o][2][r][1]:
            b = [(c, self.blocks(scheme[o][1][u], a)) for (a, u), c in term[self.side].items()]
            if self.nested or abs(b[0][1][0][0]) != abs(b[-1][1][0][0]):
                b = [(c, _lin(s)) for c, s in b]
            else:
                b = [(c * e, v) for c, s in b for e, v in s]
                if len(b) == 4:
                    b = [_signed([b[0], b[3]]), b[1], b[2]]
            slices.append(_lin(b))
        return slices


class Sums:
    def __init__(self, scheme):
        self.scheme, self.part = scheme, {}

    def add(self, o, r, m):
        for ab, c in self.scheme[o][2][r][0].items():
            old = self.part.get((o, ab))
            self.part[o, ab] = _signed([(c, m)] if old is None else [old, (c, m)])

    def result(self, i, j):
        parts = [(out[i // 2, j // 2], self.part[o, (i % 2, j % 2)])
                 for o, (out, _, _) in enumerate(self.scheme) if (i // 2, j // 2) in out]
        return _lin([(c * e, v) for c, (e, v) in reversed(parts)])


class Mxus:
    def __init__(self):
        self.load, self.target, self.stagger = [0] * 4, None, None

    def level(self, rows, lead=(0, 0, 0, 0)):
        self.target = [-(-(sum(self.load) + rows - sum(lead)) // 64) * 16 + d for d in lead]

    def __call__(self, a, b, contract=0):
        low, high, cut = min(self.load), max(self.load), 0
        if self.target:
            cut = self.target[self.load.index(low)] - low
        elif self.stagger and a.shape == (T, T) and low + T - high > self.stagger[1]:
            cut = high + self.stagger[0] - low
        if 0 < cut < a.shape[0]:
            return jnp.concatenate([self(a[:cut], b, contract), self(a[cut:], b, contract)], axis=0)
        for _ in range(0, a.shape[1], T):
            self.load[self.load.index(min(self.load))] += a.shape[0]
        return lax.dot_general(a, b, (((1,), (contract,)), ((), ())), preferred_element_type=F32)


def _after(a, v):
    n = a.shape[0]
    head = lax.select(a * a < 0, jnp.zeros(a.shape, v.dtype), v[:n])
    return head if n == v.shape[0] else jnp.concatenate([head, v[n:]], axis=0)


class Pacer:
    def __init__(self):
        self.due, self.tasks, self.products, self.done, self.lag, self.pause = [], [], [], [], 0, 0

    def spread(self, values, first, last):
        values = list(values)
        self.due += [[first + (last - first) * i // len(values), v] for i, v in enumerate(values)]

    def pace(self, steps, n, first, last, lag):
        self.drain()
        self.tasks, self.lag = [[first + (last - first) * i // n, steps] for i in range(n)], lag

    def drain(self):
        for _, steps in self.tasks:
            next(steps)
        self.tasks = []

    def note(self, product):
        self.products.append(product)
        return product

    def gate(self, operand):
        for task in self.tasks:
            task[0] -= 1
        while self.pause <= 0 and self.tasks and self.tasks[0][0] < 0:
            self.done.append(next(self.tasks.pop(0)[1]))
            self.due.append([self.lag, self.done[-1]])
        self.pause -= 1
        for d in self.due:
            d[0] -= 1
        now = [v for left, v in self.due if left < 0]
        self.due = [d for d in self.due if d[0] >= 0]
        return _after(_total(now), operand) if now else operand


def _run(*streams):
    for _, k in sorted(((i + .5) / n, k) for k, (_, n) in enumerate(streams) for i in range(n)):
        next(streams[k][0])


def _put(ref, v):
    for i in range(0, v.shape[0], T):
        part = v[i:i + T]
        pltpu.store(ref.at[i:i + part.shape[0]], part, mask=jnp.ones(part.shape, jnp.bool_))


def _fold(v):
    return jnp.sum(v.reshape(v.shape[0] // 8, 8, v.shape[1]), axis=0)


def _kernel(xT_hbm, wqkv_hbm, wo_hbm, wg_hbm, wu_hbm, wdT_hbm, outT_hbm,
            x_v, wqkv_v, wo_v, w_v, out_v, tail_v, first_v, left_v, hid_v, acc_v, wqkvT_v, wo_rows_v, sems):
    mxu, pacer = Mxus(), Pacer()

    def w_load(i, c):
        piece = max(p for p, (start, _) in enumerate(W_PIECES) if start <= c)
        return w_v[i][piece][:, pl.ds(c - W_PIECES[piece][0], 2 * T)].astype(F32)

    xn = {}

    def normalise(g):
        stats = []
        for t in range(0, 4, 2):
            def column_mean(f):
                part = None
                for i in range(0, D, 48):
                    v = _fold(f(x_v[g][i:i + 48, t * T:(t + 2) * T].astype(F32)))
                    part = v if part is None else part + v
                    yield part[:, :T] + part[:, T:]
                return jnp.sum(part, axis=0, keepdims=True) * (1.0 / D)
            mean = yield from column_mean(lambda v: v)
            var = yield from column_mean(lambda v: (v - mean) * (v - mean))
            inv = lax.rsqrt(var + 1e-5)
            stats += [(mean[:, e * T:(e + 1) * T], inv[:, e * T:(e + 1) * T]) for e in range(2)]
        for q, (mean, inv) in enumerate(stats):
            xn[g, q] = (x_v[g][:, q * T:(q + 1) * T].astype(F32) - mean) * inv
        for q in range(4):
            for i in range(0, D, 64):
                yield _fold(xn[g, q][i:i + 64])

    @functools.cache
    def x_operands(g):
        return Operands(0, lambda q, k: xn[g, q][k[0]:k[0] + k[1]])

    def store_left(g):
        products = [(o, r) for o in INPUT_ORDER for r in range(len(INPUT[o][2]))]
        for o, r in products + [p for ab in QUADS for p in _closing(INPUT, *ab)]:
            v = x_operands(g).two_levels(INPUT, o, r)
            short = T - sum(u.shape[0] for u in v)
            v = jnp.concatenate(v + [jnp.zeros((short, T), F32)] if short else v, axis=0)
            _put(left_v[g][o].at[r], pltpu.bitcast(v.astype(BF16).T, U32))
            yield pltpu.bitcast(left_v[g][o][r, T // 2 - 8:, :], F32)

    def load_left(ref):
        return pltpu.bitcast(pacer.gate(ref[...]), BF16)

    @functools.cache
    def x_one_level(g, o, a):
        return jnp.concatenate(x_operands(g).one_level(o, a), axis=0).astype(BF16)

    @functools.cache
    def gate_up_operands(n):
        w = [w_load(i, 2 * n * T) for i in range(2)]
        return Operands(1, lambda m, k: w[m // 2][k[0]:k[0] + k[1], m % 2 * T:(m % 2 + 1) * T])

    @functools.cache
    def gate_up_weight(n, o, r):
        return jnp.concatenate(gate_up_operands(n).two_levels(INPUT, o, r), axis=0).astype(BF16)

    def hidden(n, e, g, q):
        return hid_v[n % len(hid_v)][g].at[e, q]

    closing = []

    def gate_up(items, close_within=14, stops=(3,)):
        def product(sums, n, g, o, r):
            w = gate_up_weight(n, o, r)
            sums.add(o, r, pacer.note(mxu(load_left(left_v[g][o].at[r])[:, :w.shape[0]], w)))

        def close(sums, n, g, a, e):
            pacer.pause = 6
            for p in _closing(INPUT, a, e):
                product(sums, n, g, *p)
            for q in (a, a + 2):
                _put(hidden(n, e, g, q), jnp.maximum(sums.result(q, e), 0.0) * sums.result(q, e + 2))

        def steps():
            sums = {item: Sums(INPUT) for item in items}
            waiting, units = len(closing), [(o, item) for o in INPUT_ORDER for item in items]
            for i, (o, item) in enumerate(units):
                for r in range(len(INPUT[o][2])):
                    product(sums[item], *item, o, r)
                    while (r == 6 and closing
                           and len(closing) > waiting - waiting * (i + 1) // min(close_within, len(units))):
                        closing.pop(0)()
                    if r in stops:
                        yield
                if i + 1 == len(units):
                    closing.extend(functools.partial(close, sums[it], *it, *ab) for it in items for ab in QUADS)
                yield
        return steps(), 7 * (1 + len(stops)) * len(items)

    def store_first(tiles):
        for q in tiles:
            v = jnp.concatenate([xn[0, q], jnp.zeros((-D % T, T), F32)], axis=0).astype(BF16).T
            _put(first_v.at[q], pltpu.bitcast(v, U32))

    def gate_up_first():
        for q in range(4):
            for e in range(2):
                gate, up = [_total(mxu(load_left(first_v.at[q, :, k:k + T])[:, :D - k],
                                       w_v[i][0][k:min(k + T, D), e * T:(e + 1) * T])
                                   for k in range(0, D, T)) for i in range(2)]
                _put(hidden(0, e, 0, q), jnp.maximum(gate, 0.0) * up)

    @functools.cache
    def down_operands(j):
        w = [w_load(2, (4 * j + f) * T) for f in (0, 2)]
        return Operands(0, lambda d, f: w[f // 2][d * DB:(d + 1) * DB, f % 2 * T:(f % 2 + 1) * T])

    @functools.cache
    def down_weight(j, o, r):
        return down_operands(j).two_levels(DOWN, o, r)[0].astype(BF16)

    @functools.cache
    def hidden_operands(j, g):
        return Operands(1, lambda q, f: hidden(2 * j + f // 2, f % 2, g, q)[...])

    def output_product(chunks, with_heads, g, o, r):
        m = [pacer.note(mxu(down_weight(j, o, r),
                            pacer.gate(hidden_operands(j, g).two_levels(DOWN, o, r)[0]).astype(BF16), 1))
             for j in chunks]
        if with_heads:
            v = jnp.concatenate(head_operands(g).two_levels(OUTPUT, o, r), axis=0)
            m.append(mxu(attention_weight(3, o, r), v.astype(BF16)))
        if chunks and chunks[0] > 0:
            m.append(acc_v[g][o][r])
        return _total(m)

    def down(i, part=0, parts=1):
        todo = [(g, o, r) for o in OUTPUT_ORDER for r in range(7) for g in range(NG)]
        long = [t for t in todo if t[1] not in (1, 4) and t[2] not in (1, 4)]
        short = [t for t in todo if t not in long]
        todo = [t for k in range(0, len(long), 8) for t in long[k:k + 8] + short[k:k + 8]]
        todo = todo[len(todo) * part // parts:len(todo) * (part + 1) // parts]

        def steps():
            for g, o, r in todo:
                _put(acc_v[g][o].at[r], output_product((2 * i, 2 * i + 1), g == i - 1, g, o, r))
                yield
        return steps(), len(todo)

    leaving = []

    def emit(buf, g, d, q, tiles):
        rows, width = pl.ds(d * DB, DB), len(tiles) * T
        buf[...] = (jnp.concatenate(tiles, axis=1) + x_v[g][rows, pl.ds(q * T, width)].astype(F32)).astype(BF16)
        leaving.append(pltpu.make_async_copy(buf, outT_hbm.at[rows, pl.ds(g * GS + q * T, width)], sems.at[1]))
        leaving[-1].start()

    def finish(g):
        sums = Sums(OUTPUT)
        for o in OUTPUT_ORDER:
            for r in range(7):
                sums.add(o, r, output_product((NSET // 2 - 1,), g == NG - 1, g, o, r))
            yield
        for a in range(2):
            last = g == NG - 1 and a == 1
            if last:
                mxu.level(6 * DB, (64, 32, 96, 48))
            for b in range(2):
                for p in _closing(OUTPUT, a, b):
                    sums.add(*p, output_product((), True, g, *p))
                for e, f in QUADS if last else ():
                    emit(tail_v[e][b + 2 * f], g, a + 2 * e, b + 2 * f, [sums.result(a + 2 * e, b + 2 * f)])
            for d in () if last else (a, a + 2):
                emit(out_v[g][d], g, d, 0, [sums.result(d, q) for q in range(4)])
            yield

    def by_dim(ref, start):
        return jnp.concatenate([ref[pl.ds(start + d, 8, stride=DH), :] for d in range(DH)], axis=0)

    def contraction_tile(rows, t):
        start, size = (t * T, T) if t < 4 else LONE[t - 4]
        return jnp.concatenate([rows(slice(start, start + size))] * (T // size), axis=0)

    transposed = []

    def transpose_qkv():
        for columns, tiles in (((0, 2, 1, 3, 4, 6, 5, 7), (0, 2, 1, 3, 8)), ((8,), (0, 2, 1, 3, 8)),
                               (range(9, 14), (0, 2, 1, 3, 4, 5, 6, 7))):
            for t, n in itertools.product(tiles, columns):
                cols = slice(n * T, min(n * T + T, 3 * D))
                v = pltpu.bitcast(contraction_tile(lambda rows: wqkv_v[rows, cols], t), U32)
                v = pltpu.bitcast(_after(pacer.products[-1][:8, :v.shape[1]], v), BF16).T.astype(F32)
                wqkvT_v[t][cols, :] = v
                transposed.append((n, t))
                yield v[-8:]

    @functools.cache
    def wo_rows(n):
        v = wo_v[:, n * T:min(n * T + T, D)].astype(F32)
        wo_rows_v[n][...] = jnp.concatenate([v] * (T // v.shape[1]), axis=1)
        return jnp.concatenate([by_dim(wo_rows_v[n], start) for start in range(0, D, DB)], axis=0)

    @functools.cache
    def wo_transposed(n, t):
        return _after(pacer.products[-30][:8], contraction_tile(lambda rows: wo_rows(n)[rows], t)).T

    @functools.cache
    def weight_tile(part, m, t):
        if part < 3:
            start = part * D + m * DB
            assert (start // T, t) in transposed and ((start + DB - 1) // T, t) in transposed
            return by_dim(wqkvT_v[t], start)
        v = jnp.concatenate([wo_transposed(n, t) for n in (m, m + 1)], axis=0)
        return v[m * (DB - T):m * (DB - T) + DB]

    @functools.cache
    def attention_operands(part):
        return Operands(int(part < 3), nested=True, block=lambda m, k: weight_tile(
            part, m, 4 + LONE.index(k) if k in LONE else k[0] // T))

    @functools.cache
    def attention_weight(part, o, r):
        if part < 2:
            keys = [[k for _, k in term[0]] for term in ONE[o][1]]
            sums = attention_operands(part).one_level(o, r)
        else:
            scheme = INPUT if part == 2 else OUTPUT
            keys = [[k for _, u in term[0] for _, k in scheme[o][1][u][0]] for term in scheme[o][2][r][1]]
            sums = attention_operands(part).two_levels(scheme, o, r)
        lane = lax.broadcasted_iota(jnp.int32, (DB, T), 1)
        tiles = []
        for i, (ks, v) in enumerate(zip(keys, sums)):
            homes = [start % T for start, size in ks if (start, size) not in LONE]
            if not tiles or tiles[-1][2] == T:
                tiles.append([v] + (homes[:1] or [T - sum(k[0][1] for k in keys[i:])]) * 2)
            else:
                tiles[-1][0] = lax.select(lane < tiles[-1][2], tiles[-1][0], v)
            assert all(home == tiles[-1][2] for home in homes)
            tiles[-1][2] += ks[0][1]
        return jnp.concatenate([v[:, begin:end] for v, begin, end in tiles], axis=1).astype(BF16)

    qkv, heads = {}, {}

    @functools.cache
    def head_operands(g):
        rows = functools.cache(lambda q: jnp.concatenate([heads[m, 4 * g + q] for m in range(4)], axis=0))
        return Operands(1, lambda q, k: rows(q)[k[0]:k[0] + k[1]])

    def project_qk(g, m):
        for a, part in QUADS:
            c = {}
            for o, (out, _) in enumerate(ONE):
                v = mxu(attention_weight(part, o, m), x_one_level(g, o, a))
                for ij, sign in out.items():
                    c[ij] = _signed([(sign, v)] if ij not in c else [c[ij], (sign, v)])
                if o in (1, 3, 5):
                    yield
            for (i, j), v in c.items():
                qkv[part, 2 * j + m, 4 * g + 2 * i + a] = _lin([v])
            yield

    def project_v(g):
        sums = Sums(INPUT)

        def product(o, r):
            w = attention_weight(2, o, r)
            sums.add(o, r, mxu(w, load_left(left_v[g][o].at[r])[:, :w.shape[1]], 1))
        for o in INPUT_ORDER:
            for r in range(len(INPUT[o][2])):
                product(o, r)
                if r == 3:
                    yield
            yield
        for a in range(2):
            for p in _closing(INPUT, a, 0) + _closing(INPUT, a, 1):
                product(*p)
            for t, m in itertools.product((a, a + 2), range(4)):
                qkv[2, m, 4 * g + t] = sums.result(t, m)
            yield

    def windows():
        lane = lax.broadcasted_iota(jnp.int32, (8 * DIMS, T), 1)
        wraps = [lane >= T - DIL * w for w in range(WIN)]
        dims = [slice(8 * d, 8 * (d + DIMS)) for d in range(0, DH, DIMS)]

        def shifted(part, m, t, rows):
            here = qkv[part, m, t][rows]
            before = qkv[part, m, t - 1][rows] if t else jnp.broadcast_to(here[:, :1], here.shape)
            before = _after(jnp.concatenate([pacer.products[-1][:8] + pacer.done[-2]] * DIMS, axis=0), before)
            return [here] + [pltpu.roll(lax.select(wraps[w], before, here), DIL * w, 1) for w in range(1, WIN)]
        for g in range(NG):
            probs = {}
            for m, t in itertools.product((0, 2, 1, 3), range(4 * g, 4 * g + 4)):
                logits = None
                for rows in dims:
                    if logits is not None:
                        yield _fold(logits)
                    q = qkv[0, m, t][rows]
                    p = jnp.concatenate([q * k for k in shifted(1, m, t, rows)], axis=0)
                    p = jnp.sum(p.reshape(WIN, DIMS, 8, T), axis=1).reshape(8 * WIN, T)
                    logits = p if logits is None else logits + p
                logits = (logits * DH ** -0.5).reshape(WIN, 8, T)
                if t == 0:
                    offset = DIL * lax.broadcasted_iota(jnp.int32, logits.shape, 0)
                    logits = jnp.where(lax.broadcasted_iota(jnp.int32, logits.shape, 2) >= offset, logits, -1e9)
                e = jnp.exp(logits - jnp.max(logits, axis=0, keepdims=True))
                inv = 1.0 / jnp.sum(e, axis=0)
                probs[m, t] = e * inv
                yield inv
            for (m, t), p in probs.items():
                p = [jnp.concatenate([p[w]] * DIMS, axis=0) for w in range(WIN)]
                o = []
                for rows in dims:
                    o.append(_total(a * v for a, v in zip(p, shifted(2, m, t, rows))))
                    if rows == dims[-1]:
                        heads[m, t] = jnp.concatenate(o, axis=0)
                    yield _fold(o[-1])

    def copies(i):
        x = lambda g: [(xT_hbm.at[:, pl.ds(g * GS, GS)], x_v[g])]
        w = lambda which, pieces: [((wg_hbm, wu_hbm, wdT_hbm)[k].at[:, pl.ds(*W_PIECES[p])], w_v[k][p])
                                   for p in pieces for k in which]
        pairs = (x(0), w((0, 1), [0]), w((0, 1), [1]), w((0, 1), [2]) + x(1),
                 w((0, 1), [3]) + x(2) + x(3) + w((2,), [0, 1]),
                 [(wqkv_hbm, wqkv_v)] + w((2,), [2, 3]) + w((0, 1), [4]),
                 [(wo_hbm, wo_v)] + w((2,), [4]) + w((0, 1, 2), [5]))[i]
        return [pltpu.make_async_copy(src, dst, sems.at[i % 2]) for src, dst in pairs]

    def arrive(i, then=None, lead=(0, 0, 0, 0)):
        if closing:
            mxu.level(4 * T, lead)
            closing.pop(0)()
            closing.pop(0)()
            mxu.target = None
        for c in copies(i):
            c.wait()
        for c in copies(then) if then else ():
            c.start()
        pacer.due.clear()

    for c in copies(0) + copies(1):
        c.start()
    arrive(0, 2)
    list(normalise(0))
    store_first((0, 1))
    arrive(1, 3)
    store_first((2, 3))
    left = store_left(0)
    pacer.spread(itertools.islice(left, 52), 37, 80)
    gate_up_first()
    arrive(2)
    list(left)
    _run(gate_up([(1, 0)]))
    arrive(3, 4)
    mxu.stagger = 48, 80
    pacer.spread(normalise(1), 0, 52)
    _run(gate_up([(2, 0)]))
    pacer.spread(itertools.islice(store_left(1), 4, None), 0, 162)
    _run(gate_up([(1, 1), (2, 1), (0, 1)]))
    arrive(4, 5)
    pacer.spread(normalise(2), 0, 110)
    _run(gate_up([(3, 0), (3, 1)]))
    pacer.spread(itertools.islice(store_left(2), 4, None), 0, 216)
    left = store_left(3)
    pacer.spread(itertools.chain(normalise(3), itertools.islice(left, 8)), 100, 216)
    _run(gate_up([(n, 2) for n in range(4)]))
    arrive(5, 6)
    mxu.stagger = None
    pacer.spread(left, 0, 180)
    pacer.pace(transpose_qkv(), 85, 4, 215, 16)
    _run(gate_up([(n, 3) for n in range(4)]), (itertools.chain([None] * 26, project_qk(0, 0)), 26 + 16))

    softmax = windows()
    for n in range(4, NSET - 2):
        if n == 8:
            arrive(6, lead=(48, 32, 16, 0))
            mxu.stagger = 32, 96
        g, stage = divmod(n - 3, 3)
        pacer.pace(softmax, ((12, 11, 9)[stage] - 4 * (n == 4)) * DH // DIMS, 0,
                   335 - 50 * (n == 4) - 30 * (n == 7), 24)
        project = [] if g == NG else [(project_qk(g, stage) if stage < 2 else project_v(g), 8)]
        for half in range(2):
            i, part = divmod(2 * n - 9 + half, 8)
            _run(gate_up([(n, 2 * half), (n, 2 * half + 1)], stops=(1, 3, 5)),
                 *[down(i, part, 8)] * (i >= 0), *project)

    pacer.pace(softmax, 4 * DH // DIMS, 0, 450, 24)
    steps, n = gate_up([(NSET - 2, 0), (NSET - 1, 0)], close_within=3)
    _run((steps, 8), down(2, 7, 8))
    _run((steps, n - 8), down(3))
    for g in range(1, NG):
        steps, n = gate_up([(NSET - 2, g), (NSET - 1, g)], close_within=6)
        result = finish(g - 1)
        _run((steps, n // 2))
        _run((steps, n // 2), (result, 9 - (g == NG - 1)))
    pacer.drain()
    while closing:
        closing.pop(0)()
    next(result)
    list(finish(NG - 1))
    for c in leaving:
        c.wait()


@jax.jit
def pallas_parallel_sum__sliding_local_dilated__glu_gated_reglu__prompt_kernel(
    A_x: jax.Array,
    A_wqkv: jax.Array,
    A_wo: jax.Array,
    B_x: jax.Array,
    B_W_gate: jax.Array,
    B_W_up: jax.Array,
    B_W_down: jax.Array,
):
    del B_x
    vmem, hbm = pltpu.VMEM, pl.BlockSpec(memory_space=pltpu.HBM)
    outT = pl.pallas_call(
        _kernel,
        in_specs=[hbm] * 6,
        out_specs=hbm,
        out_shape=jax.ShapeDtypeStruct((D, S), BF16),
        scratch_shapes=[
            [vmem((D, GS), BF16)] * NG,
            vmem((D, 3 * D), BF16),
            vmem((D, D), BF16),
            [[vmem((D, n), BF16) for _, n in W_PIECES]] * 3,
            [[vmem((DB, GS), BF16)] * 4] * NG,
            [[vmem((DB, T), BF16)] * 4] * 2,
            vmem((4, T // 2, 5 * T), U32),
            [[vmem((len(i), T // 2, T), U32) for _, _, i in INPUT]] * NG,
            [[vmem((2, 4, T, T), F32)] * NG] * 9,
            [[vmem((7, DB, T), F32)] * 7] * NG,
            [vmem((3 * D, T), F32)] * 9,
            [vmem((D, T), F32)] * 5,
            pltpu.SemaphoreType.DMA((2,)),
        ],
        compiler_params=pltpu.CompilerParams(vmem_limit_bytes=120 << 20),
    )(A_x.reshape(S, D).T, A_wqkv, A_wo, B_W_gate, B_W_up, B_W_down.T)
    return outT.T.reshape(1, S, D)
```

```python
import functools
import itertools

import jax
import jax.numpy as jnp
from jax import lax
from jax.experimental import pallas as pl
from jax.experimental.pallas import tpu as pltpu

F32, BF16, U32 = jnp.float32, jnp.bfloat16, jnp.uint32

S, D, F = 2048, 576, 4608
DH, WIN, DIL = 18, 8, 2
T = 128
GS = 4 * T
NG = S // GS
DB = D // 4
NSET = F // (2 * T)
DIMS = 3
W_PIECES = ((0, 256), (256, 256), (512, 256), (768, 256), (1024, 1024), (2048, F - 2048))
QUADS = ((0, 0), (0, 1), (1, 0), (1, 1))


OUTS = {
    "m1": {(0, 0): 1, (1, 1): 1}, "m2": {(1, 0): 1, (1, 1): -1}, "m4": {(0, 0): 1, (1, 0): 1},
    "m3": {(0, 1): 1, (1, 1): 1}, "m5": {(0, 1): 1, (0, 0): -1}, "m6": {(1, 1): 1}, "m7": {(0, 0): 1},
    "c12": {(0, 1): 1}, "c21": {(1, 0): 1}, "x": {(0, 1): 1, (1, 0): 1},
    "e1": {(0, 0): 1, (1, 0): -1}, "e2": {(0, 1): 1, (1, 1): -1},
}


def _strassen(p, q):
    return {
        "m1": ({(0, p): 1, (1, q): 1}, {(0, p): 1, (1, q): 1}),
        "m2": ({(1, p): 1, (1, q): 1}, {(0, p): 1}),
        "m4": ({(1, q): 1}, {(0, q): 1, (0, p): -1}),
        "m3": ({(0, p): 1}, {(1, p): 1, (1, q): -1}),
        "m5": ({(0, p): 1, (0, q): 1}, {(1, q): 1}),
        "m6": ({(1, p): 1, (0, p): -1}, {(0, p): 1, (1, p): 1}),
        "m7": ({(0, q): 1, (1, q): -1}, {(0, q): 1, (1, q): 1}),
    }


def _strassen_mirrored(p, q):
    return {
        "x": ({(0, p): 1, (1, q): 1}, {(1, p): 1, (0, q): 1}),
        "m2": ({(1, p): -1, (1, q): -1}, {(1, p): 1}),
        "m3": ({(1, q): 1}, {(1, q): 1, (1, p): -1}),
        "m4": ({(0, p): 1}, {(0, p): 1, (0, q): -1}),
        "m5": ({(0, p): -1, (0, q): -1}, {(0, q): 1}),
        "c21": ({(1, p): 1, (0, p): -1}, {(0, p): 1, (1, p): 1}),
        "c12": ({(0, q): 1, (1, q): -1}, {(0, q): 1, (1, q): 1}),
    }


def _plain(k):
    return {name: ({(i, k): 1}, {(j, k): 1}) for name, (i, j) in zip(("m7", "c12", "c21", "m6"), QUADS)}


def _single(k, variant):
    u0, u1, n1 = {(0, k): 1}, {(1, k): 1}, {(1, k): -1}
    add, sub = {(0, k): 1, (1, k): 1}, {(0, k): 1, (1, k): -1}
    half_add, half_sub = {(0, k): .5, (1, k): .5}, {(0, k): .5, (1, k): -.5}
    return (
        {"e1": (n1, u0), "e2": (n1, u1), "m7": (add, add), "m5": (add, u1)},
        {"e1": (u0, u0), "e2": (u0, u1), "m6": (add, add), "m2": (add, u0)},
        {"e1": (half_sub, u0), "e2": (half_sub, u1), "m4": (half_add, u0), "m3": (half_add, u1)},
        {"e1": (n1, u0), "e2": (u0, u1), "m1": (add, u1), "m7": (add, sub)},
    )[variant]


def _merge(parts):
    return [(out, [p[name] for p in parts if name in p])
            for name, out in OUTS.items() if any(name in p for p in parts)]


def _two_levels(outer):
    scheme = []
    for o, (out, terms) in enumerate(outer):
        n = len(terms)
        if o >= 7:
            inner = _merge([_plain(u) for u in range(n)])
        elif n == 5:
            inner = _merge([_strassen(0, 2), _single(3, 0), _single(4, 1), _single(1, 2)])
        elif n == 3:
            cut = lambda term: tuple({key: c for key, c in form.items() if key[1] < 3} for form in term)
            inner = [(ab, [t for t in map(cut, ts) if all(t)])
                     for ab, ts in _merge([_strassen(0, 3), _strassen(1, 2)])]
        else:
            inner = _merge([_strassen(u, u + n // 2) for u in range(n // 2)])
        if 3 <= o < 7:
            inner = [({(a, 1 - b): c for (a, b), c in ab.items()},
                      [(left, {(1 - b, u): c for (b, u), c in right.items()}) for left, right in ts])
                     for ab, ts in inner]
        scheme.append((out, terms, inner))
    return scheme


def _pair(start, size):
    return (start, size), (start + 2 * T, size)


LONE = ((224, 32), (480, 32), (512, 32), (544, 32), (512, 64))
ONE = _merge([_strassen(*_pair(0, 64)), _strassen(*_pair(64, 64)), _strassen_mirrored(*_pair(128, 64)),
              _plain(LONE[4]), _strassen(*_pair(192, 64))])
OUTPUT = _two_levels(ONE)
INPUT = _two_levels(_merge([_strassen(*_pair(0, 96)), _strassen(*_pair(96, 32)), _strassen(*_pair(128, 96))]
                           + [_single(LONE[v], v) for v in range(4)]))
DOWN = _two_levels(_merge([_strassen(0, 2), _strassen(1, 3)]))
INPUT_ORDER, OUTPUT_ORDER = (1, 5, 3, 0, 4, 2, 6), (3, 2, 0, 1, 5, 4, 6)


def _closing(scheme, a, b):
    return [(o, r) for o in range(7, len(scheme)) for r in range(4) if (a, b) in scheme[o][2][r][0]]


def _total(vs):
    vs = list(vs)
    while len(vs) > 1:
        vs = [a + b for a, b in zip(vs[::2], vs[1::2])] + vs[len(vs) // 2 * 2:]
    return vs[0]


def _signed(pairs):
    first = next((i for i, (c, _) in enumerate(pairs) if c > 0), 0)
    scale, v = pairs[first]
    for c, t in pairs[:first] + pairs[first + 1:]:
        v = v + t if c == scale else v - t
    return scale, v


def _lin(pairs):
    c, v = _signed(pairs)
    return v if c == 1 else v * c


class Operands:
    def __init__(self, side, block, nested=False):
        self.side, self.block, self.nested = side, functools.cache(block), nested

    def blocks(self, term, a):
        return [(c, self.block(2 * i + a, k)) for (i, k), c in term[self.side].items()]

    def one_level(self, o, a):
        return [_lin(self.blocks(term, a)) for term in ONE[o][1]]

    def two_levels(self, scheme, o, r):
        slices = []
        for term in scheme[o][2][r][1]:
            b = [(c, self.blocks(scheme[o][1][u], a)) for (a, u), c in term[self.side].items()]
            if self.nested or abs(b[0][1][0][0]) != abs(b[-1][1][0][0]):
                b = [(c, _lin(s)) for c, s in b]
            else:
                b = [(c * e, v) for c, s in b for e, v in s]
                if len(b) == 4:
                    b = [_signed([b[0], b[3]]), b[1], b[2]]
            slices.append(_lin(b))
        return slices


class Sums:
    def __init__(self, scheme):
        self.scheme, self.part = scheme, {}

    def add(self, o, r, m):
        for ab, c in self.scheme[o][2][r][0].items():
            old = self.part.get((o, ab))
            self.part[o, ab] = _signed([(c, m)] if old is None else [old, (c, m)])

    def result(self, i, j):
        parts = [(out[i // 2, j // 2], self.part[o, (i % 2, j % 2)])
                 for o, (out, _, _) in enumerate(self.scheme) if (i // 2, j // 2) in out]
        return _lin([(c * e, v) for c, (e, v) in reversed(parts)])


class Mxus:
    def __init__(self):
        self.load, self.target, self.stagger = [0] * 4, None, None

    def level(self, rows, lead=(0, 0, 0, 0)):
        self.target = [-(-(sum(self.load) + rows - sum(lead)) // 64) * 16 + d for d in lead]

    def __call__(self, a, b, contract=0):
        low, high, cut = min(self.load), max(self.load), 0
        if self.target:
            cut = self.target[self.load.index(low)] - low
        elif self.stagger and a.shape == (T, T) and low + T - high > self.stagger[1]:
            cut = high + self.stagger[0] - low
        if 0 < cut < a.shape[0]:
            return jnp.concatenate([self(a[:cut], b, contract), self(a[cut:], b, contract)], axis=0)
        for _ in range(0, a.shape[1], T):
            self.load[self.load.index(min(self.load))] += a.shape[0]
        return lax.dot_general(a, b, (((1,), (contract,)), ((), ())), preferred_element_type=F32)


def _after(a, v):
    n = a.shape[0]
    head = lax.select(a * a < 0, jnp.zeros(a.shape, v.dtype), v[:n])
    return head if n == v.shape[0] else jnp.concatenate([head, v[n:]], axis=0)


class Pacer:
    def __init__(self):
        self.due, self.tasks, self.products, self.done, self.lag, self.pause = [], [], [], [], 0, 0

    def spread(self, values, first, last):
        values = list(values)
        self.due += [[first + (last - first) * i // len(values), v] for i, v in enumerate(values)]

    def pace(self, steps, n, first, last, lag):
        self.drain()
        self.tasks, self.lag = [[first + (last - first) * i // n, steps] for i in range(n)], lag

    def drain(self):
        for _, steps in self.tasks:
            next(steps)
        self.tasks = []

    def note(self, product):
        self.products.append(product)
        return product

    def gate(self, operand):
        for task in self.tasks:
            task[0] -= 1
        while self.pause <= 0 and self.tasks and self.tasks[0][0] < 0:
            self.done.append(next(self.tasks.pop(0)[1]))
            self.due.append([self.lag, self.done[-1]])
        self.pause -= 1
        for d in self.due:
            d[0] -= 1
        now = [v for left, v in self.due if left < 0]
        self.due = [d for d in self.due if d[0] >= 0]
        return _after(_total(now), operand) if now else operand


def _run(*streams):
    for _, k in sorted(((i + .5) / n, k) for k, (_, n) in enumerate(streams) for i in range(n)):
        next(streams[k][0])


def _put(ref, v):
    for i in range(0, v.shape[0], T):
        part = v[i:i + T]
        pltpu.store(ref.at[i:i + part.shape[0]], part, mask=jnp.ones(part.shape, jnp.bool_))


def _fold(v):
    return jnp.sum(v.reshape(v.shape[0] // 8, 8, v.shape[1]), axis=0)


def _kernel(xT_hbm, wqkv_hbm, wo_hbm, wg_hbm, wu_hbm, wdT_hbm, outT_hbm,
            x_v, wqkv_v, wo_v, w_v, out_v, tail_v, first_v, left_v, hid_v, acc_v, wqkvT_v, wo_rows_v, sems):
    mxu, pacer = Mxus(), Pacer()

    def w_load(i, c):
        piece = max(p for p, (start, _) in enumerate(W_PIECES) if start <= c)
        return w_v[i][piece][:, pl.ds(c - W_PIECES[piece][0], 2 * T)].astype(F32)

    xn = {}

    def normalise(g):
        stats = []
        for t in range(0, 4, 2):
            def column_mean(f):
                part = None
                for i in range(0, D, 48):
                    v = _fold(f(x_v[g][i:i + 48, t * T:(t + 2) * T].astype(F32)))
                    part = v if part is None else part + v
                    yield part[:, :T] + part[:, T:]
                return jnp.sum(part, axis=0, keepdims=True) * (1.0 / D)
            mean = yield from column_mean(lambda v: v)
            var = yield from column_mean(lambda v: (v - mean) * (v - mean))
            inv = lax.rsqrt(var + 1e-5)
            stats += [(mean[:, e * T:(e + 1) * T], inv[:, e * T:(e + 1) * T]) for e in range(2)]
        for q, (mean, inv) in enumerate(stats):
            xn[g, q] = (x_v[g][:, q * T:(q + 1) * T].astype(F32) - mean) * inv
        for q in range(4):
            for i in range(0, D, 64):
                yield _fold(xn[g, q][i:i + 64])

    @functools.cache
    def x_operands(g):
        return Operands(0, lambda q, k: xn[g, q][k[0]:k[0] + k[1]])

    def store_left(g):
        products = [(o, r) for o in INPUT_ORDER for r in range(len(INPUT[o][2]))]
        for o, r in products + [p for ab in QUADS for p in _closing(INPUT, *ab)]:
            v = x_operands(g).two_levels(INPUT, o, r)
            short = T - sum(u.shape[0] for u in v)
            v = jnp.concatenate(v + [jnp.zeros((short, T), F32)] if short else v, axis=0)
            _put(left_v[g][o].at[r], pltpu.bitcast(v.astype(BF16).T, U32))
            yield pltpu.bitcast(left_v[g][o][r, T // 2 - 8:, :], F32)

    @functools.cache
    def stored_left(g, o, r):
        v = left_v[g][o][r]
        return v, pltpu.bitcast(v, BF16)

    def load_left(g, o, r):
        words, v = stored_left(g, o, r)
        gated = pacer.gate(words)
        return v if gated is words else pltpu.bitcast(gated, BF16)

    @functools.cache
    def x_one_level(g, o, a):
        return jnp.concatenate(x_operands(g).one_level(o, a), axis=0).astype(BF16)

    @functools.cache
    def gate_up_operands(n):
        w = [w_load(i, 2 * n * T) for i in range(2)]
        return Operands(1, lambda m, k: w[m // 2][k[0]:k[0] + k[1], m % 2 * T:(m % 2 + 1) * T])

    @functools.cache
    def gate_up_weight(n, o, r):
        return jnp.concatenate(gate_up_operands(n).two_levels(INPUT, o, r), axis=0).astype(BF16)

    def hidden(n, e, g, q):
        return hid_v[n % len(hid_v)][g].at[e, q]

    closing = []

    def gate_up(items, close_within=14, stops=(3,)):
        def product(sums, n, g, o, r):
            w = gate_up_weight(n, o, r)
            sums.add(o, r, pacer.note(mxu(load_left(g, o, r)[:, :w.shape[0]], w)))

        def close(sums, n, g, a, e):
            pacer.pause = 6
            for p in _closing(INPUT, a, e):
                product(sums, n, g, *p)
            for q in (a, a + 2):
                _put(hidden(n, e, g, q), jnp.maximum(sums.result(q, e), 0.0) * sums.result(q, e + 2))

        def steps():
            sums = {item: Sums(INPUT) for item in items}
            waiting, units = len(closing), [(o, item) for o in INPUT_ORDER for item in items]
            for i, (o, item) in enumerate(units):
                for r in range(len(INPUT[o][2])):
                    product(sums[item], *item, o, r)
                    while (r == 6 and closing
                           and len(closing) > waiting - waiting * (i + 1) // min(close_within, len(units))):
                        closing.pop(0)()
                    if r in stops:
                        yield
                if i + 1 == len(units):
                    closing.extend(functools.partial(close, sums[it], *it, *ab) for it in items for ab in QUADS)
                yield
        return steps(), 7 * (1 + len(stops)) * len(items)

    def store_first(tiles):
        for q in tiles:
            v = jnp.concatenate([xn[0, q], jnp.zeros((-D % T, T), F32)], axis=0).astype(BF16).T
            _put(first_v.at[q], pltpu.bitcast(v, U32))

    def gate_up_first():
        for q in range(4):
            for e in range(2):
                gate, up = [_total(mxu(pltpu.bitcast(pacer.gate(first_v[q, :, k:k + T]), BF16)[:, :D - k],
                                       w_v[i][0][k:min(k + T, D), e * T:(e + 1) * T])
                                   for k in range(0, D, T)) for i in range(2)]
                _put(hidden(0, e, 0, q), jnp.maximum(gate, 0.0) * up)

    @functools.cache
    def down_operands(j):
        w = [w_load(2, (4 * j + f) * T) for f in (0, 2)]
        return Operands(0, lambda d, f: w[f // 2][d * DB:(d + 1) * DB, f % 2 * T:(f % 2 + 1) * T])

    @functools.cache
    def down_weight(j, o, r):
        return down_operands(j).two_levels(DOWN, o, r)[0].astype(BF16)

    @functools.cache
    def hidden_operands(j, g):
        return Operands(1, lambda q, f: hidden(2 * j + f // 2, f % 2, g, q)[...])

    def output_product(chunks, with_heads, g, o, r):
        m = [pacer.note(mxu(down_weight(j, o, r),
                            pacer.gate(hidden_operands(j, g).two_levels(DOWN, o, r)[0]).astype(BF16), 1))
             for j in chunks]
        if with_heads:
            v = jnp.concatenate(head_operands(g).two_levels(OUTPUT, o, r), axis=0)
            m.append(mxu(attention_weight(3, o, r), v.astype(BF16)))
        if chunks and chunks[0] > 0:
            m.append(acc_v[g][o][r])
        return _total(m)

    def down(i, part=0, parts=1):
        todo = [(g, o, r) for o in OUTPUT_ORDER for r in range(7) for g in range(NG)]
        long = [t for t in todo if t[1] not in (1, 4) and t[2] not in (1, 4)]
        short = [t for t in todo if t not in long]
        todo = [t for k in range(0, len(long), 8) for t in long[k:k + 8] + short[k:k + 8]]
        todo = todo[len(todo) * part // parts:len(todo) * (part + 1) // parts]

        def steps():
            for g, o, r in todo:
                _put(acc_v[g][o].at[r], output_product((2 * i, 2 * i + 1), g == i - 1, g, o, r))
                yield
        return steps(), len(todo)

    leaving = []

    def emit(buf, g, d, q, tiles):
        rows, width = pl.ds(d * DB, DB), len(tiles) * T
        buf[...] = (jnp.concatenate(tiles, axis=1) + x_v[g][rows, pl.ds(q * T, width)].astype(F32)).astype(BF16)
        leaving.append(pltpu.make_async_copy(buf, outT_hbm.at[rows, pl.ds(g * GS + q * T, width)], sems.at[1]))
        leaving[-1].start()

    def finish(g):
        sums = Sums(OUTPUT)
        for o in OUTPUT_ORDER:
            for r in range(7):
                sums.add(o, r, output_product((NSET // 2 - 1,), g == NG - 1, g, o, r))
            yield
        for a in range(2):
            last = g == NG - 1 and a == 1
            if last:
                mxu.level(6 * DB, (64, 32, 96, 48))
            for b in range(2):
                for p in _closing(OUTPUT, a, b):
                    sums.add(*p, output_product((), True, g, *p))
                for e, f in QUADS if last else ():
                    emit(tail_v[e][b + 2 * f], g, a + 2 * e, b + 2 * f, [sums.result(a + 2 * e, b + 2 * f)])
            for d in () if last else (a, a + 2):
                emit(out_v[g][d], g, d, 0, [sums.result(d, q) for q in range(4)])
            yield

    def by_dim(ref, start):
        return jnp.concatenate([ref[pl.ds(start + d, 8, stride=DH), :] for d in range(DH)], axis=0)

    def contraction_tile(rows, t):
        start, size = (t * T, T) if t < 4 else LONE[t - 4]
        return jnp.concatenate([rows(slice(start, start + size))] * (T // size), axis=0)

    transposed = []

    def transpose_qkv():
        for columns, tiles in (((0, 2, 1, 3, 4, 6, 5, 7), (0, 2, 1, 3, 8)), ((8,), (0, 2, 1, 3, 8)),
                               (range(9, 14), (0, 2, 1, 3, 4, 5, 6, 7))):
            for t, n in itertools.product(tiles, columns):
                cols = slice(n * T, min(n * T + T, 3 * D))
                v = pltpu.bitcast(contraction_tile(lambda rows: wqkv_v[rows, cols], t), U32)
                v = pltpu.bitcast(_after(pacer.products[-1][:8, :v.shape[1]], v), BF16).T.astype(F32)
                wqkvT_v[t][cols, :] = v
                transposed.append((n, t))
                yield v[-8:]

    @functools.cache
    def wo_rows(n):
        v = wo_v[:, n * T:min(n * T + T, D)].astype(F32)
        wo_rows_v[n][...] = jnp.concatenate([v] * (T // v.shape[1]), axis=1)
        return jnp.concatenate([by_dim(wo_rows_v[n], start) for start in range(0, D, DB)], axis=0)

    @functools.cache
    def wo_transposed(n, t):
        return _after(pacer.products[-30][:8], contraction_tile(lambda rows: wo_rows(n)[rows], t)).T

    @functools.cache
    def weight_tile(part, m, t):
        if part < 3:
            start = part * D + m * DB
            assert (start // T, t) in transposed and ((start + DB - 1) // T, t) in transposed
            return by_dim(wqkvT_v[t], start)
        v = jnp.concatenate([wo_transposed(n, t) for n in (m, m + 1)], axis=0)
        return v[m * (DB - T):m * (DB - T) + DB]

    @functools.cache
    def attention_operands(part):
        return Operands(int(part < 3), nested=True, block=lambda m, k: weight_tile(
            part, m, 4 + LONE.index(k) if k in LONE else k[0] // T))

    @functools.cache
    def attention_weight(part, o, r):
        if part < 2:
            keys = [[k for _, k in term[0]] for term in ONE[o][1]]
            sums = attention_operands(part).one_level(o, r)
        else:
            scheme = INPUT if part == 2 else OUTPUT
            keys = [[k for _, u in term[0] for _, k in scheme[o][1][u][0]] for term in scheme[o][2][r][1]]
            sums = attention_operands(part).two_levels(scheme, o, r)
        lane = lax.broadcasted_iota(jnp.int32, (DB, T), 1)
        tiles = []
        for i, (ks, v) in enumerate(zip(keys, sums)):
            homes = [start % T for start, size in ks if (start, size) not in LONE]
            if not tiles or tiles[-1][2] == T:
                tiles.append([v] + (homes[:1] or [T - sum(k[0][1] for k in keys[i:])]) * 2)
            else:
                tiles[-1][0] = lax.select(lane < tiles[-1][2], tiles[-1][0], v)
            assert all(home == tiles[-1][2] for home in homes)
            tiles[-1][2] += ks[0][1]
        return jnp.concatenate([v[:, begin:end] for v, begin, end in tiles], axis=1).astype(BF16)

    qkv, heads = {}, {}

    @functools.cache
    def head_operands(g):
        rows = functools.cache(lambda q: jnp.concatenate([heads[m, 4 * g + q] for m in range(4)], axis=0))
        return Operands(1, lambda q, k: rows(q)[k[0]:k[0] + k[1]])

    def project_qk(g, m):
        for a, part in QUADS:
            c = {}
            for o, (out, _) in enumerate(ONE):
                v = mxu(attention_weight(part, o, m), x_one_level(g, o, a))
                for ij, sign in out.items():
                    c[ij] = _signed([(sign, v)] if ij not in c else [c[ij], (sign, v)])
                if o in (1, 3, 5):
                    yield
            for (i, j), v in c.items():
                qkv[part, 2 * j + m, 4 * g + 2 * i + a] = _lin([v])
            yield

    def project_v(g):
        sums = Sums(INPUT)

        def product(o, r):
            w = attention_weight(2, o, r)
            sums.add(o, r, mxu(w, load_left(g, o, r)[:, :w.shape[1]], 1))
        for o in INPUT_ORDER:
            for r in range(len(INPUT[o][2])):
                product(o, r)
                if r == 3:
                    yield
            yield
        for a in range(2):
            for p in _closing(INPUT, a, 0) + _closing(INPUT, a, 1):
                product(*p)
            for t, m in itertools.product((a, a + 2), range(4)):
                qkv[2, m, 4 * g + t] = sums.result(t, m)
            yield

    def windows():
        shape = (WIN - 1, 8 * DIMS, T)
        wraps = lax.broadcasted_iota(jnp.int32, shape, 2) >= T - DIL * (1 + lax.broadcasted_iota(jnp.int32, shape, 0))
        dims = [slice(8 * d, 8 * (d + DIMS)) for d in range(0, DH, DIMS)]

        def shifted(part, m, t, rows):
            here = qkv[part, m, t][rows]
            before = qkv[part, m, t - 1][rows] if t else jnp.broadcast_to(here[:, :1], here.shape)
            before = _after(jnp.concatenate([pacer.products[-1][:8] + pacer.done[-2]] * DIMS, axis=0), before)
            v = lax.select(wraps, jnp.broadcast_to(before, shape), jnp.broadcast_to(here, shape))
            return jnp.concatenate([here[None], pltpu.roll(v, DIL, 2, stride=DIL, stride_axis=0)], axis=0)
        for g in range(NG):
            probs = {}
            for m, t in itertools.product((0, 2, 1, 3), range(4 * g, 4 * g + 4)):
                logits = None
                for rows in dims:
                    if logits is not None:
                        yield _fold(logits)
                    p = qkv[0, m, t][rows] * shifted(1, m, t, rows)
                    p = jnp.sum(p.reshape(WIN, DIMS, 8, T), axis=1).reshape(8 * WIN, T)
                    logits = p if logits is None else logits + p
                logits = (logits * DH ** -0.5).reshape(WIN, 8, T)
                if t == 0:
                    offset = DIL * lax.broadcasted_iota(jnp.int32, logits.shape, 0)
                    logits = jnp.where(lax.broadcasted_iota(jnp.int32, logits.shape, 2) >= offset, logits, -1e9)
                e = jnp.exp(logits - jnp.max(logits, axis=0, keepdims=True))
                inv = 1.0 / jnp.sum(e, axis=0)
                probs[m, t] = e * inv
                yield inv
            for (m, t), p in probs.items():
                p = jnp.concatenate([p] * DIMS, axis=1)
                o = []
                for rows in dims:
                    o.append(jnp.sum(p * shifted(2, m, t, rows), axis=0))
                    if rows == dims[-1]:
                        heads[m, t] = jnp.concatenate(o, axis=0)
                    yield _fold(o[-1])

    def copies(i):
        x = lambda g: [(xT_hbm.at[:, pl.ds(g * GS, GS)], x_v[g])]
        w = lambda which, pieces: [((wg_hbm, wu_hbm, wdT_hbm)[k].at[:, pl.ds(*W_PIECES[p])], w_v[k][p])
                                   for p in pieces for k in which]
        pairs = (x(0), w((0, 1), [0]), w((0, 1), [1]), w((0, 1), [2]) + x(1),
                 w((0, 1), [3]) + x(2) + x(3) + w((2,), [0, 1]),
                 [(wqkv_hbm, wqkv_v)] + w((2,), [2, 3]) + w((0, 1), [4]),
                 [(wo_hbm, wo_v)] + w((2,), [4]) + w((0, 1, 2), [5]))[i]
        return [pltpu.make_async_copy(src, dst, sems.at[i % 2]) for src, dst in pairs]

    def arrive(i, then=None, lead=(0, 0, 0, 0)):
        if closing:
            mxu.level(4 * T, lead)
            closing.pop(0)()
            closing.pop(0)()
            mxu.target = None
        for c in copies(i):
            c.wait()
        for c in copies(then) if then else ():
            c.start()
        pacer.due.clear()
        stored_left.cache_clear()

    for c in copies(0) + copies(1):
        c.start()
    arrive(0, 2)
    list(normalise(0))
    store_first((0, 1))
    arrive(1, 3)
    store_first((2, 3))
    left = store_left(0)
    pacer.spread(itertools.islice(left, 52), 37, 80)
    gate_up_first()
    arrive(2)
    list(left)
    _run(gate_up([(1, 0)]))
    arrive(3, 4)
    mxu.stagger = 48, 80
    pacer.spread(normalise(1), 0, 52)
    _run(gate_up([(2, 0)]))
    pacer.spread(itertools.islice(store_left(1), 4, None), 0, 162)
    _run(gate_up([(1, 1), (2, 1), (0, 1)]))
    arrive(4, 5)
    pacer.spread(normalise(2), 0, 110)
    _run(gate_up([(3, 0), (3, 1)]))
    pacer.spread(itertools.islice(store_left(2), 4, None), 0, 216)
    left = store_left(3)
    pacer.spread(itertools.chain(normalise(3), itertools.islice(left, 8)), 100, 216)
    _run(gate_up([(n, 2) for n in range(4)], close_within=20))
    arrive(5, 6)
    mxu.stagger = None
    pacer.spread(left, 0, 180)
    pacer.pace(transpose_qkv(), 85, 4, 215, 16)
    _run(gate_up([(n, 3) for n in range(4)], close_within=20),
         (itertools.chain([None] * 26, project_qk(0, 0)), 26 + 16))

    softmax = windows()
    for n in range(4, NSET - 2):
        if n == 8:
            arrive(6, lead=(48, 32, 16, 0))
            mxu.stagger = 32, 96
        g, stage = divmod(n - 3, 3)
        pacer.pace(softmax, ((12, 11, 9)[stage] - 4 * (n == 4)) * DH // DIMS, 120 * (n == 4),
                   335 - 50 * (n == 4) - 30 * (n == 7), 24)
        project = [] if g == NG else [(project_qk(g, stage) if stage < 2 else project_v(g), 8)]
        for half in range(2):
            i, part = divmod(2 * n - 9 + half, 8)
            _run(gate_up([(n, 2 * half), (n, 2 * half + 1)], stops=(1, 3, 5)),
                 *[down(i, part, 8)] * (i >= 0), *project)

    pacer.pace(softmax, 4 * DH // DIMS, 0, 450, 24)
    steps, n = gate_up([(NSET - 2, 0), (NSET - 1, 0)], close_within=3)
    _run((steps, 8), down(2, 7, 8))
    _run((steps, n - 8), down(3))
    for g in range(1, NG):
        steps, n = gate_up([(NSET - 2, g), (NSET - 1, g)], close_within=6)
        result = finish(g - 1)
        _run((steps, n // 2))
        _run((steps, n // 2), (result, 9 - (g == NG - 1)))
    pacer.drain()
    while closing:
        closing.pop(0)()
    next(result)
    list(finish(NG - 1))
    for c in leaving:
        c.wait()


@jax.jit
def pallas_parallel_sum__sliding_local_dilated__glu_gated_reglu__prompt_kernel(
    A_x: jax.Array,
    A_wqkv: jax.Array,
    A_wo: jax.Array,
    B_x: jax.Array,
    B_W_gate: jax.Array,
    B_W_up: jax.Array,
    B_W_down: jax.Array,
):
    del B_x
    vmem, hbm = pltpu.VMEM, pl.BlockSpec(memory_space=pltpu.HBM)
    outT = pl.pallas_call(
        _kernel,
        in_specs=[hbm] * 6,
        out_specs=hbm,
        out_shape=jax.ShapeDtypeStruct((D, S), BF16),
        scratch_shapes=[
            [vmem((D, GS), BF16)] * NG,
            vmem((D, 3 * D), BF16),
            vmem((D, D), BF16),
            [[vmem((D, n), BF16) for _, n in W_PIECES]] * 3,
            [[vmem((DB, GS), BF16)] * 4] * NG,
            [[vmem((DB, T), BF16)] * 4] * 2,
            vmem((4, T // 2, 5 * T), U32),
            [[vmem((len(i), T // 2, T), U32) for _, _, i in INPUT]] * NG,
            [[vmem((2, 4, T, T), F32)] * NG] * 9,
            [[vmem((7, DB, T), F32)] * 7] * NG,
            [vmem((3 * D, T), F32)] * 9,
            [vmem((D, T), F32)] * 5,
            pltpu.SemaphoreType.DMA((2,)),
        ],
        compiler_params=pltpu.CompilerParams(vmem_limit_bytes=120 << 20),
    )(A_x.reshape(S, D).T, A_wqkv, A_wo, B_W_gate, B_W_up, B_W_down.T)
    return outT.T.reshape(1, S, D)
```
